```python
import os as _os
_os.environ.setdefault("JAX_PLATFORMS", "cpu")
import jax
import jax.numpy as jnp

def _softmax(x, axis=-1):
    return jax.nn.softmax(x, axis=axis)
def _gelu(x):
    return jax.nn.gelu(x, approximate=True)
def _silu(x):
    return jax.nn.silu(x)
def _sigmoid(x):
    return jax.nn.sigmoid(x)
def _layernorm(x, axis=-1, eps=1e-5):
    m = jnp.mean(x, axis=axis, keepdims=True)
    v = jnp.var(x, axis=axis, keepdims=True)
    return (x - m) / jnp.sqrt(v + eps)
def _scatter_add(tgt, idx, src, axis=0):
    return tgt.at[idx].add(src)
def _segment_sum(src, seg, n):
    return jax.ops.segment_sum(src, seg, n)
class _Rng:
    def __init__(self, key):
        self._k = key
    def _next(self):
        self._k, sub = jax.random.split(self._k)
        return sub
    def normal(self, shape):
        return jax.random.normal(self._next(), shape, dtype=jnp.bfloat16)
    def randint(self, lo, hi, shape):
        return jax.random.randint(self._next(), shape, lo, hi, dtype=jnp.int32)
    def uniform(self, shape, lo=0.0, hi=1.0):
        return jax.random.uniform(self._next(), shape, jnp.bfloat16, lo, hi)
    def permutation(self, n):
        return jax.random.permutation(self._next(), n)


kernel_name = 'concat_heads__sliding_local_dilated__sliding_block__prompt'

def setup_inputs():
    _rng = _Rng(jax.random.key(int.from_bytes(__import__("os").urandom(4), "little")))
    _w = (lambda a: (lambda t: t.astype(jnp.bfloat16) if jnp.issubdtype(t.dtype, jnp.floating) else t)(jnp.asarray(a)))
    def _A_setup():
        B, S, D = 1, 2048, 1024
        return {
            "x": _w((lambda *s: _rng.normal(s) * 0.2)(B, S, D)),
            "wqkv": _w((lambda *s: _rng.normal(s) * 0.2)(D, 3 * D)),
            "wo": _w((lambda *s: _rng.normal(s) * 0.05)(D, D)),
        }
    _A_in = _A_setup()

    def _B_setup():
        B, S, D = 1, 2048, 1024
        return {
            "x": _w((lambda *s: _rng.normal(s) * 0.2)(B, S, D)),
            "wqkv": _w((lambda *s: _rng.normal(s) * 0.2)(D, 3 * D)),
            "wo": _w((lambda *s: _rng.normal(s) * 0.05)(D, D)),
        }
    _B_in = _B_setup()

    return {
        "A_x": _A_in["x"],
        "A_wqkv": _A_in["wqkv"],
        "A_wo": _A_in["wo"],
        "B_x": _B_in["x"],
        "B_wqkv": _B_in["wqkv"],
        "B_wo": _B_in["wo"],
    }

def reference(A_x, A_wqkv, A_wo, B_x, B_wqkv, B_wo):
    def _A_ref(x, wqkv, wo):
        B, S, D = x.shape
        H = 32; Dh = D // H
        W, dil = 8, 2
        qkv = (lambda x, *d: x.transpose(*d))((x @ wqkv).reshape(B, S, 3, H, Dh), 2, 0, 3, 1, 4)
        q, k, v = qkv[0], qkv[1], qkv[2]
        scale = Dh ** -0.5
        pos = jnp.arange(S)
        off = jnp.arange(W) * dil
        idx = pos[:, None] - off[None, :]
        mask = idx >= 0
        idx_c = jnp.where(mask, idx, 0).reshape(-1)
        kg = k[:, :, idx_c, :].reshape(B, H, S, W, Dh)
        vg = v[:, :, idx_c, :].reshape(B, H, S, W, Dh)
        logits = jnp.einsum("bhsd,bhswd->bhsw", q, kg) * scale
        logits = jnp.where(mask[None, None, :, :], logits, -1e9)
        attn = _softmax(logits, axis=-1)
        o = jnp.einsum("bhsw,bhswd->bhsd", attn, vg)
        return (lambda x, *d: x.transpose(*d))(o, 0, 2, 1, 3).reshape(B, S, D) @ wo

    def _B_ref(x, wqkv, wo):
        B, S, D = x.shape
        H = 32; Dh = D // H; W = 256
        qkv = (lambda x, *d: x.transpose(*d))((x @ wqkv).reshape(B, S, 3, H, Dh), 2, 0, 3, 1, 4)
        q, k, v = qkv[0], qkv[1], qkv[2]
        scores = jnp.einsum("bhqd,bhkd->bhqk", q, k) * (Dh ** -0.5)
        idx = jnp.arange(S)
        mask = (idx[:, None] - idx[None, :] >= 0) & (idx[:, None] - idx[None, :] < W)
        scores = jnp.where(mask[None, None], scores, -1e9)
        p = _softmax(scores, axis=-1)
        o = jnp.einsum("bhqk,bhkd->bhqd", p, v)
        return (lambda x, *d: x.transpose(*d))(o, 0, 2, 1, 3).reshape(B, S, D) @ wo

    a = _A_ref(A_x, A_wqkv, A_wo)
    b = _B_ref(B_x, B_wqkv, B_wo)
    return jnp.concatenate([a, b], axis=-1)
```

```python
import jax
import jax.numpy as jnp
from jax import lax
from jax.experimental import pallas as pl
from jax.experimental.pallas import tpu as pltpu

S, D, H, DH = 2048, 1024, 32, 32
T = 128
NT = S // T
WIN = 256
TAPS, DIL = 8, 2
SCALE = DH ** -0.5 * 1.4426950408889634
NEG = -1e30
QS = 64
NBLK = WIN // QS + 1
CH = 16
AHEAD = 2
OSPLIT = 8

bf, f32, u32 = jnp.bfloat16, jnp.float32, jnp.uint32

ORDER = {
    "PTO": "qB2 r sB0 fA0 r r pB0 r".split(),
    "PT": "qB2 pB0 r fA0 sB1 r r r".split(),
    "TO": "r sB0 r pB-1 r r fA0 qB2".split(),
    "O": "r".split(),
}
A_CHAIN = {"PTO": 1, "PT": 1, "TO": 2}
N_ACC = {"PTO": 8, "PT": 4, "TO": 8}


def _dot(a, b):
    return jnp.dot(a, b, preferred_element_type=f32)


def _dot_nt(a, b):
    return lax.dot_general(a, b, (((1,), (1,)), ((), ())), preferred_element_type=f32)


def _recip(x):
    r = pl.reciprocal(x, approx=True)
    return r * (2.0 - x * r)


def _kernel(ax_h, aw_h, awo_h, bx_h, bw_h, bwo_h, o_h,
            aw, awo, bw, bwo, awT32, awo32, bw32, bwT32, bwo32, xva, xvb, o_v,
            aqT, akT, avT, aoT, bq, bk, bvT, boT, zref, wsem, xsem, osem):
    def w_copies(g):
        sem = wsem.at[g % 3 if isinstance(g, int) else lax.rem(g, 3)]
        res = []
        for src, dst in ((aw_h, aw), (bw_h, bw)):
            for t in range(3):
                lo = t * D + 128 * g
                c = pl.ds(lo if isinstance(g, int) else pl.multiple_of(lo, 128), 128)
                res.append(pltpu.make_async_copy(src.at[:, c], dst.at[:, c], sem))
        return res

    def wo_copies():
        return [pltpu.make_async_copy(awo_h, awo, wsem.at[3]), pltpu.make_async_copy(bwo_h, bwo, wsem.at[3])]

    def x_copies(t):
        if isinstance(t, int):
            rows, slot = pl.ds(t * T, T), t % 3
        else:
            rows, slot = pl.ds(pl.multiple_of(t * T, T), T), lax.rem(t, 3)
        return [pltpu.make_async_copy(src.at[rows, :], dst.at[slot], xsem.at[slot])
                for src, dst in ((ax_h, xva), (bx_h, xvb))]

    def o_copy(s):
        if isinstance(s, int):
            rows, slot = pl.ds((s - 2) * T, T), s % 2
        else:
            rows, slot = pl.ds(pl.multiple_of((s - 2) * T, T), T), lax.rem(s, 2)
        return pltpu.make_async_copy(o_v.at[slot], o_h.at[rows, :], osem.at[slot])

    def o_last(lo, n):
        slot = (NT + 1) % 2
        return pltpu.make_async_copy(o_v.at[slot, :, pl.ds(lo, n)],
                                     o_h.at[pl.ds((NT - 1) * T, T), pl.ds(lo, n)], osem.at[slot])

    def start(copies):
        for c in copies:
            c.start()

    def wait(copies):
        for c in copies:
            c.wait()

    def first_step():
        start(x_copies(0) + x_copies(1) + w_copies(0))
        bk[0:2 * T, :] = jnp.zeros((2 * T, D), bf)
        bvT[0] = jnp.zeros((D, T), bf)
        bvT[1] = jnp.zeros((D, T), bf)
        akT[0] = jnp.zeros((D, T), bf)
        avT[0] = jnp.zeros((D, T), bf)
        zref[...] = jnp.zeros((8, T), u32)
        wait(x_copies(0) + x_copies(1))
        for g in range(1, AHEAD):
            start(w_copies(g))

        def body(g, carry):
            wait(w_copies(g))
            pl.when(g + AHEAD < 8)(lambda: start(w_copies(g + AHEAD)))
            pl.when(g + AHEAD == 7)(lambda: start(wo_copies()))
            pl.when(g == 3)(lambda: start(x_copies(2)))
            lo = pl.multiple_of(128 * g, 128)
            cols = pl.ds(lo, 128)

            def chunk(ref, t, ref32=None):
                c = pl.ds(pl.multiple_of(t * D + lo, 128), 128)
                v = ref[:, c]
                if ref32 is not None:
                    ref32[:, c] = pltpu.bitcast(v, u32)
                return v

            xa = xva[0:2].reshape(2 * T, D)
            xb = xvb[0:2].reshape(2 * T, D)
            wt = chunk(bw, 2).T
            bwT32[pl.ds(pl.multiple_of(64 * g, 64), 64), :] = pltpu.bitcast(wt, u32)
            for t, dst, off in ((0, aqT, 0), (1, akT, 1), (2, avT, 1)):
                wta = chunk(aw, t).T
                awT32[pl.ds(pl.multiple_of(t * (D // 2) + 64 * g, 64), 64), :] = pltpu.bitcast(wta, u32)
                r = _dot_nt(wta, xa)
                if t == 0:
                    r = r * SCALE
                for u in range(2):
                    dst[u + off, cols, :] = r[:, u * T:(u + 1) * T].astype(bf)
            bq[0:2 * T, cols] = (_dot(xb, chunk(bw, 0, bw32)) * SCALE).astype(bf)
            bk[2 * T:4 * T, cols] = _dot(xb, chunk(bw, 1, bw32)).astype(bf)
            r = _dot_nt(wt, xb)
            for u in range(2):
                bvT[u + 2, cols, :] = r[:, u * T:(u + 1) * T].astype(bf)
            return carry

        lax.fori_loop(0, 8, body, 0)

    def step(s, kind):
        doP, doT, doO = "P" in kind, "T" in kind, "O" in kind
        sp, J, Jo = s + 1, s - 1, s - 2
        if doO:
            pl.when(s >= 4)(lambda: o_copy(s - 2).wait())
            o = o_v.at[lax.rem(s, 2)]
        if doP:
            pl.when(sp + 1 < NT)(lambda: start(x_copies(sp + 1)))
            wait(x_copies(sp))
            xa = xva[lax.rem(sp, 3)]
            xb = xvb[lax.rem(sp, 3)]
            r0 = pl.multiple_of(sp * T, T)

        def proj_a(lo, n):
            r = _dot_nt(pltpu.bitcast(awT32[lo // 2:(lo + n) // 2, :], bf), xa)
            t, c = divmod(lo, D)
            if t == 0:
                aqT[sp, c:c + n, :] = (r * SCALE).astype(bf)
            elif t == 1:
                akT[sp + 1, c:c + n, :] = r.astype(bf)
            else:
                avT[sp + 1, c:c + n, :] = r.astype(bf)

        def proj_b(lo, n):
            r = _dot(xb, pltpu.bitcast(bw32[:, lo:lo + n], bf))
            t, c = divmod(lo, D)
            if t == 0:
                bq[pl.ds(r0, T), c:c + n] = (r * SCALE).astype(bf)
            else:
                bk[pl.ds(pl.multiple_of(r0 + 2 * T, T), T), c:c + n] = r.astype(bf)

        def proj_bv(lo, n):
            bvT[sp + 2, lo:lo + n, :] = _dot_nt(pltpu.bitcast(bwT32[lo // 2:(lo + n) // 2, :], bf), xb).astype(bf)

        if doT:
            rq = lax.broadcasted_iota(jnp.int32, (QS, T), 0)
            lq = lax.broadcasted_iota(jnp.int32, (QS, T), 1)
            le = rq <= (lq % QS)
            half = lq // QS
            head_of_lane = lax.broadcasted_iota(jnp.int32, (1, T), 1) // DH
            rJ = pl.multiple_of(J * T, T)
            nacc = N_ACC[kind]

            def before_start(c, b):
                return jnp.where(J * 2 + c + b >= NBLK - 1, 0.0, NEG)

        def qk_b(g):
            q = bq[pl.ds(rJ, T), 128 * g:128 * (g + 1)].astype(f32)
            res = []
            for c in range(2):
                k = bk[pl.ds(pl.multiple_of(rJ + QS * c, QS), WIN + QS), 128 * g:128 * (g + 1)]
                w = [jnp.where(head_of_lane == 2 * p + (L - c) % 2, q[QS * c:QS * (c + 1)], 0.0)
                     for p in range(2) for L in range(2)]
                sc = _dot_nt(k, jnp.concatenate(w, axis=0).astype(bf))
                res.append([sc[:, p * T:(p + 1) * T] for p in range(2)])
            return res

        def softmax_b(scores):
            outs = []
            for p in range(2):
                blocks, sums = [], []
                for c in range(2):
                    sh = scores[c][p]
                    srcs = [jnp.where(le, sh[WIN:WIN + QS], sh[0:QS] + before_start(c, 0))]
                    srcs += [sh[QS * b:QS * (b + 1)] + before_start(c, b) for b in range(1, NBLK - 1)]
                    mx = srcs[0]
                    for z in srcs[1:]:
                        mx = jnp.maximum(mx, z)
                    m = jnp.max(mx, axis=0, keepdims=True)
                    accs, k, probs = [None] * nacc, 0, []
                    for src in srcs:
                        parts = []
                        for r0_ in range(0, QS, CH):
                            pc = jnp.exp2(src[r0_:r0_ + CH] - m)
                            for r in range(0, CH, 8):
                                a = accs[k % nacc]
                                accs[k % nacc] = pc[r:r + 8] if a is None else a + pc[r:r + 8]
                                k += 1
                            parts.append(pc)
                        probs.append(jnp.concatenate(parts, axis=0))
                    while len(accs) > 1:
                        accs = [accs[i] + accs[i + 1] for i in range(0, len(accs), 2)]
                    sums.append(jnp.sum(accs[0], axis=0, keepdims=True))
                    blocks.append(probs + [probs[0]])
                for e in range(2):
                    frames, masks, full = [], [], []
                    for F in range(3 * T // QS):
                        val = msk = None
                        n, dense = 0, True
                        for c in range(2):
                            b = F - c
                            if not 0 <= b < NBLK:
                                continue
                            n += 1
                            mine = half == (e + c) % 2
                            val = blocks[c][b] if val is None else jnp.where(mine, blocks[c][b], val)
                            if b == 0:
                                ok, dense = mine & ~le, False
                            elif b == NBLK - 1:
                                ok, dense = mine & le, False
                            else:
                                ok = mine
                            msk = ok if msk is None else msk | ok
                        frames.append(val)
                        masks.append(msk)
                        full.append(dense and n == 2)
                    tiles = []
                    for t in range(3):
                        v = jnp.concatenate(frames[2 * t:2 * t + 2], axis=0)
                        if not all(full[2 * t:2 * t + 2]):
                            v = jnp.where(jnp.concatenate(masks[2 * t:2 * t + 2], axis=0), v, 0.0)
                        tiles.append(v)
                    pT = jnp.concatenate(tiles, axis=0).astype(bf)
                    outs.append((pT, _recip(jnp.where(half[0:1] == (e + 1) % 2, sums[1], sums[0]))))
            return outs

        def pv_b(g, probs):
            for hh in range(4):
                rows = slice(DH * (4 * g + hh), DH * (4 * g + hh + 1))
                v = jnp.concatenate([bvT[J + t, rows, :] for t in range(3)], axis=1)
                ov = _dot(v, probs[hh][0]) * probs[hh][1]
                if hh % 2:
                    ov = pltpu.roll(ov, QS, 1)
                boT[J, rows, :] = ov.astype(bf)

        if doT:
            lane16 = lax.broadcasted_iota(jnp.int32, (DH // 2, T), 1)
            lane1 = lax.broadcasted_iota(jnp.int32, (1, T), 1)
            tap_ok = [None] + [(lane1 >= DIL * w) | (J >= 1) for w in range(1, TAPS)]
            zero = zref[0:1, :]
            done = {}

        def taps(ref, rows, after):
            cur = pltpu.bitcast(ref[J + 1, rows, :], u32)
            prv = pltpu.bitcast(ref[J, rows, :], u32)
            if after is not None:
                z = pltpu.bitcast(after, u32) & zero
                cur, prv = cur | z, prv | z
            res = []
            for w in range(TAPS):
                sh = DIL * w
                z = cur if w == 0 else jnp.where(lane16 < sh, pltpu.roll(prv, sh, 1), pltpu.roll(cur, sh, 1))
                res.append(pltpu.bitcast(z, bf).astype(f32))
            return res

        def attn_a(g):
            for h in range(4 * g, 4 * g + 4):
                rows = slice(DH * h, DH * (h + 1))
                q = aqT[J, rows, :].astype(f32)
                logits = []
                for w, kf in enumerate(taps(akT, rows, done.get(h - A_CHAIN[kind]))):
                    l = jnp.sum(q * kf, axis=0, keepdims=True)
                    logits.append(l if w == 0 else jnp.where(tap_ok[w], l, NEG))
                m = logits[0]
                for l in logits[1:]:
                    m = jnp.maximum(m, l)
                ps = [jnp.exp2(l - m) for l in logits]
                tot = ps[0]
                for p in ps[1:]:
                    tot = tot + p
                r = _recip(tot)
                acc = None
                for p, vf in zip(ps, taps(avT, rows, logits[0])):
                    t = (p * r) * vf
                    acc = t if acc is None else acc + t
                aoT[J, rows, :] = acc.astype(bf)
                done[h] = acc[0:1]

        if doO:
            oa = aoT[Jo].T
            ob = boT[Jo].T

        def out_a(lo, n):
            o[:, lo:lo + n] = _dot(oa, pltpu.bitcast(awo32[:, lo:lo + n], bf)).astype(bf)

        def out_b(lo, n):
            o[:, D + lo:D + lo + n] = _dot(ob, pltpu.bitcast(bwo32[:, lo:lo + n], bf)).astype(bf)

        lists = []
        if doP:
            lists += [[(fn, lo, 128) for lo in range(0, n * D, 128)] for fn, n in ((proj_a, 3), (proj_b, 2), (proj_bv, 1))]
        if kind == "O":
            piece, seq = 2 * D // OSPLIT, []
            for c in range(0, 2 * D, 128):
                seq.append((out_a, c, 128) if c < D else (out_b, c - D, 128))
                if (c + 128) % piece == 0:
                    seq.append((lambda lo, n: o_last(lo, n).start(), c + 128 - piece, piece))
            lists.append(seq)
        elif doO:
            lists += [[(fn, lo, 128) for lo in range(0, D, 128)] for fn in (out_a, out_b)]
        order = ORDER[kind]
        nr = order.count("r")
        slots = [[] for _ in range(nr * 8)]
        for frac, task in sorted((((i + 0.5) / len(l), t) for l in lists for i, t in enumerate(l)), key=lambda z: z[0]):
            slots[min(int(frac * nr * 8), nr * 8 - 1)].append(task)
        offs = [0] + [int(t[2:]) for t in order if t != "r"]
        scores, probs = {}, {}
        for i in range(-max(offs), 8 - min(offs)):
            k = 0
            for tok in order:
                if tok == "r":
                    if 0 <= i < 8:
                        for fn, lo, n in slots[nr * i + k]:
                            fn(lo, n)
                    k += 1
                    continue
                g = i + int(tok[2:])
                if not 0 <= g < 8:
                    continue
                if tok[:2] == "qB":
                    scores[g] = qk_b(g)
                elif tok[:2] == "sB":
                    probs[g] = softmax_b(scores.pop(g))
                elif tok[:2] == "pB":
                    pv_b(g, probs.pop(g))
                else:
                    attn_a(g)
        if kind == "PT":
            wait(wo_copies())
            awo32[...] = pltpu.bitcast(awo[...], u32)
            bwo32[...] = pltpu.bitcast(bwo[...], u32)
        if doO and kind != "O":
            o_copy(s).start()

    first_step()
    step(jnp.int32(1), "PT")
    lax.fori_loop(2, NT - 1, lambda s, c: (step(s, "PTO"), c)[1], 0)
    lax.fori_loop(NT - 1, NT + 1, lambda s, c: (step(s, "TO"), c)[1], 0)
    step(jnp.int32(NT + 1), "O")
    o_copy(NT).wait()
    for lo in range(0, 2 * D, 2 * D // OSPLIT):
        o_last(lo, 2 * D // OSPLIT).wait()


@jax.jit
def pallas_concat_heads__sliding_local_dilated__sliding_block__prompt_kernel(
    A_x: jax.Array,
    A_wqkv: jax.Array,
    A_wo: jax.Array,
    B_x: jax.Array,
    B_wqkv: jax.Array,
    B_wo: jax.Array,
):
    hbm = pl.BlockSpec(memory_space=pl.ANY)
    vmem = pltpu.VMEM
    out = pl.pallas_call(
        _kernel,
        in_specs=[hbm] * 6,
        out_specs=hbm,
        out_shape=jax.ShapeDtypeStruct((S, 2 * D), bf),
        scratch_shapes=[
            vmem((D, 3 * D), bf), vmem((D, D), bf), vmem((D, 3 * D), bf), vmem((D, D), bf),
            vmem((3 * D // 2, D), u32), vmem((D // 2, D), u32),
            vmem((D // 2, 2 * D), u32), vmem((D // 2, D), u32), vmem((D // 2, D), u32),
            vmem((3, T, D), bf), vmem((3, T, D), bf), vmem((2, T, 2 * D), bf),
            vmem((NT, D, T), bf), vmem((NT + 1, D, T), bf), vmem((NT + 1, D, T), bf),
            vmem((NT, D, T), bf),
            vmem((S, D), bf), vmem((S + 2 * T, D), bf),
            vmem((NT + 2, D, T), bf), vmem((NT, D, T), bf),
            vmem((8, T), u32),
            pltpu.SemaphoreType.DMA((4,)), pltpu.SemaphoreType.DMA((3,)), pltpu.SemaphoreType.DMA((2,)),
        ],
        compiler_params=pltpu.CompilerParams(vmem_limit_bytes=100 * 1024 * 1024),
    )(A_x[0], A_wqkv, A_wo, B_x[0], B_wqkv, B_wo)
    return out[None]
```

```python
import jax
import jax.numpy as jnp
from jax import lax
from jax.experimental import pallas as pl
from jax.experimental.pallas import tpu as pltpu

S, D, H, DH = 2048, 1024, 32, 32
T = 128
NT = S // T
WIN = 256
TAPS, DIL = 8, 2
SCALE = DH ** -0.5 * 1.4426950408889634
NEG = -1e30
QS = 64
NBLK = WIN // QS + 1
CH = 16
AHEAD = 2
OSPLIT = 8

bf, f32, u32 = jnp.bfloat16, jnp.float32, jnp.uint32

ORDER = {
    "PTO": "qB1 r sB0 fA0 r r pB0 r".split(),
    "PT": "r sB1 qB2 pB0 r fA0 r r".split(),
    "TO": "r sB1 r pB-1 r qB2 r fA0".split(),
    "O": "r".split(),
}
A_CHAIN = {"PTO": 1, "PT": 1, "TO": 2}
N_ACC = {"PTO": 4, "PT": 4, "TO": 8}


def _dot(a, b):
    return jnp.dot(a, b, preferred_element_type=f32)


def _dot_nt(a, b):
    return lax.dot_general(a, b, (((1,), (1,)), ((), ())), preferred_element_type=f32)


def _recip(x):
    fn = pltpu.reciprocal if hasattr(pltpu, "reciprocal") else pl.reciprocal
    return fn(x, approx=True)


def _kernel(ax_h, aw_h, awo_h, bx_h, bw_h, bwo_h, o_h,
            aw, awo, bw, bwo, awT32, awo32, bw32, bwT32, bwo32, xva, xvb, o_v,
            aqT, akT, avT, aoT, bq, bk, bvT, boT, zref, wsem, xsem, osem):
    def w_copies(g):
        sem = wsem.at[g % 3 if isinstance(g, int) else lax.rem(g, 3)]
        res = []
        for src, dst in ((aw_h, aw), (bw_h, bw)):
            for t in range(3):
                lo = t * D + 128 * g
                c = pl.ds(lo if isinstance(g, int) else pl.multiple_of(lo, 128), 128)
                res.append(pltpu.make_async_copy(src.at[:, c], dst.at[:, c], sem))
        return res

    def wo_copies():
        return [pltpu.make_async_copy(awo_h, awo, wsem.at[3]), pltpu.make_async_copy(bwo_h, bwo, wsem.at[3])]

    def x_copies(t):
        if isinstance(t, int):
            rows, slot = pl.ds(t * T, T), t % 3
        else:
            rows, slot = pl.ds(pl.multiple_of(t * T, T), T), lax.rem(t, 3)
        return [pltpu.make_async_copy(src.at[rows, :], dst.at[slot], xsem.at[slot])
                for src, dst in ((ax_h, xva), (bx_h, xvb))]

    def o_copy(s):
        if isinstance(s, int):
            rows, slot = pl.ds((s - 2) * T, T), s % 2
        else:
            rows, slot = pl.ds(pl.multiple_of((s - 2) * T, T), T), lax.rem(s, 2)
        return pltpu.make_async_copy(o_v.at[slot], o_h.at[rows, :], osem.at[slot])

    def o_last(lo, n):
        slot = (NT + 1) % 2
        return pltpu.make_async_copy(o_v.at[slot, :, pl.ds(lo, n)],
                                     o_h.at[pl.ds((NT - 1) * T, T), pl.ds(lo, n)], osem.at[slot])

    def start(copies):
        for c in copies:
            c.start()

    def wait(copies):
        for c in copies:
            c.wait()

    def first_step():
        start(x_copies(0) + x_copies(1) + w_copies(0))
        bk[0:2 * T, :] = jnp.zeros((2 * T, D), bf)
        bvT[0] = jnp.zeros((D, T), bf)
        bvT[1] = jnp.zeros((D, T), bf)
        akT[0] = jnp.zeros((D, T), bf)
        avT[0] = jnp.zeros((D, T), bf)
        zref[...] = jnp.zeros((8, T), u32)
        wait(x_copies(0) + x_copies(1))
        for g in range(1, AHEAD):
            start(w_copies(g))

        def body(g, carry):
            wait(w_copies(g))
            pl.when(g + AHEAD < 8)(lambda: start(w_copies(g + AHEAD)))
            pl.when(g + AHEAD == 7)(lambda: start(wo_copies()))
            pl.when(g == 3)(lambda: start(x_copies(2)))
            lo = pl.multiple_of(128 * g, 128)
            cols = pl.ds(lo, 128)

            def chunk(ref, t, ref32=None):
                c = pl.ds(pl.multiple_of(t * D + lo, 128), 128)
                v = ref[:, c]
                if ref32 is not None:
                    ref32[:, c] = pltpu.bitcast(v, u32)
                return v

            xa = xva[0:2].reshape(2 * T, D)
            xb = xvb[0:2].reshape(2 * T, D)
            wt = chunk(bw, 2).T
            bwT32[pl.ds(pl.multiple_of(64 * g, 64), 64), :] = pltpu.bitcast(wt, u32)
            for t, dst, off in ((0, aqT, 0), (1, akT, 1), (2, avT, 1)):
                wta = chunk(aw, t).T
                awT32[pl.ds(pl.multiple_of(t * (D // 2) + 64 * g, 64), 64), :] = pltpu.bitcast(wta, u32)
                r = _dot_nt(wta, xa)
                if t == 0:
                    r = r * SCALE
                for u in range(2):
                    dst[u + off, cols, :] = r[:, u * T:(u + 1) * T].astype(bf)
            bq[0:2 * T, cols] = (_dot(xb, chunk(bw, 0, bw32)) * SCALE).astype(bf)
            bk[2 * T:4 * T, cols] = _dot(xb, chunk(bw, 1, bw32)).astype(bf)
            r = _dot_nt(wt, xb)
            for u in range(2):
                bvT[u + 2, cols, :] = r[:, u * T:(u + 1) * T].astype(bf)
            return carry

        lax.fori_loop(0, 8, body, 0)

    def step(s, kind):
        doP, doT, doO = "P" in kind, "T" in kind, "O" in kind
        sp, J, Jo = s + 1, s - 1, s - 2
        if doO:
            pl.when(s >= 4)(lambda: o_copy(s - 2).wait())
            o = o_v.at[lax.rem(s, 2)]
        if doP:
            pl.when(sp + 1 < NT)(lambda: start(x_copies(sp + 1)))
            wait(x_copies(sp))
            xa = xva[lax.rem(sp, 3)]
            xb = xvb[lax.rem(sp, 3)]
            r0 = pl.multiple_of(sp * T, T)

        def proj_a(lo, n):
            r = _dot_nt(pltpu.bitcast(awT32[lo // 2:(lo + n) // 2, :], bf), xa)
            t, c = divmod(lo, D)
            if t == 0:
                aqT[sp, c:c + n, :] = (r * SCALE).astype(bf)
            elif t == 1:
                akT[sp + 1, c:c + n, :] = r.astype(bf)
            else:
                avT[sp + 1, c:c + n, :] = r.astype(bf)

        def proj_b(lo, n):
            r = _dot(xb, pltpu.bitcast(bw32[:, lo:lo + n], bf))
            t, c = divmod(lo, D)
            if t == 0:
                bq[pl.ds(r0, T), c:c + n] = (r * SCALE).astype(bf)
            else:
                bk[pl.ds(pl.multiple_of(r0 + 2 * T, T), T), c:c + n] = r.astype(bf)

        def proj_bv(lo, n):
            bvT[sp + 2, lo:lo + n, :] = _dot_nt(pltpu.bitcast(bwT32[lo // 2:(lo + n) // 2, :], bf), xb).astype(bf)

        if doT:
            rq = lax.broadcasted_iota(jnp.int32, (QS, T), 0)
            lq = lax.broadcasted_iota(jnp.int32, (QS, T), 1)
            le = rq <= (lq % QS)
            half = lq // QS
            head_of_lane = lax.broadcasted_iota(jnp.int32, (1, T), 1) // DH
            rJ = pl.multiple_of(J * T, T)
            nacc = N_ACC[kind]

            def before_start(c, b):
                return jnp.where(J * 2 + c + b >= NBLK - 1, 0.0, NEG)

        def qk_b(g):
            q = bq[pl.ds(rJ, T), 128 * g:128 * (g + 1)].astype(f32)
            res = []
            for c in range(2):
                k = bk[pl.ds(pl.multiple_of(rJ + QS * c, QS), WIN + QS), 128 * g:128 * (g + 1)]
                w = [jnp.where(head_of_lane == 2 * p + (L - c) % 2, q[QS * c:QS * (c + 1)], 0.0)
                     for p in range(2) for L in range(2)]
                sc = _dot_nt(k, jnp.concatenate(w, axis=0).astype(bf))
                res.append([sc[:, p * T:(p + 1) * T] for p in range(2)])
            return res

        def softmax_b(scores):
            outs = []
            for p in range(2):
                blocks, sums = [], []
                for c in range(2):
                    sh = scores[c][p]
                    srcs = [jnp.where(le, sh[WIN:WIN + QS], sh[0:QS] + before_start(c, 0))]
                    srcs += [sh[QS * b:QS * (b + 1)] + before_start(c, b) for b in range(1, NBLK - 1)]
                    mx = srcs[0]
                    for z in srcs[1:]:
                        mx = jnp.maximum(mx, z)
                    m = jnp.max(mx, axis=0, keepdims=True)
                    accs, k, probs = [None] * nacc, 0, []
                    for src in srcs:
                        parts = []
                        for r0_ in range(0, QS, CH):
                            pc = jnp.exp2(src[r0_:r0_ + CH] - m)
                            for r in range(0, CH, 8):
                                a = accs[k % nacc]
                                accs[k % nacc] = pc[r:r + 8] if a is None else a + pc[r:r + 8]
                                k += 1
                            parts.append(pc)
                        probs.append(jnp.concatenate(parts, axis=0))
                    while len(accs) > 1:
                        accs = [accs[i] + accs[i + 1] for i in range(0, len(accs), 2)]
                    sums.append(jnp.sum(accs[0], axis=0, keepdims=True))
                    blocks.append(probs + [probs[0]])
                for e in range(2):
                    frames, masks, full = [], [], []
                    for F in range(3 * T // QS):
                        val = msk = None
                        n, dense = 0, True
                        for c in range(2):
                            b = F - c
                            if not 0 <= b < NBLK:
                                continue
                            n += 1
                            mine = half == (e + c) % 2
                            val = blocks[c][b] if val is None else jnp.where(mine, blocks[c][b], val)
                            if b == 0:
                                ok, dense = mine & ~le, False
                            elif b == NBLK - 1:
                                ok, dense = mine & le, False
                            else:
                                ok = mine
                            msk = ok if msk is None else msk | ok
                        frames.append(val)
                        masks.append(msk)
                        full.append(dense and n == 2)
                    tiles = []
                    for t in range(3):
                        v = jnp.concatenate(frames[2 * t:2 * t + 2], axis=0)
                        if not all(full[2 * t:2 * t + 2]):
                            v = jnp.where(jnp.concatenate(masks[2 * t:2 * t + 2], axis=0), v, 0.0)
                        tiles.append(v)
                    pT = jnp.concatenate(tiles, axis=0).astype(bf)
                    outs.append((pT, _recip(jnp.where(half[0:1] == (e + 1) % 2, sums[1], sums[0]))))
            return outs

        def pv_b(g, probs):
            for hh in range(4):
                rows = slice(DH * (4 * g + hh), DH * (4 * g + hh + 1))
                v = jnp.concatenate([bvT[J + t, rows, :] for t in range(3)], axis=1)
                ov = _dot(v, probs[hh][0]) * probs[hh][1]
                if hh % 2:
                    ov = pltpu.roll(ov, QS, 1)
                boT[J, rows, :] = ov.astype(bf)

        if doT:
            lane16 = lax.broadcasted_iota(jnp.int32, (DH // 2, T), 1)
            lane1 = lax.broadcasted_iota(jnp.int32, (1, T), 1)
            tap_ok = [None] + [(lane1 >= DIL * w) | (J >= 1) for w in range(1, TAPS)]
            zero = zref[0:1, :]
            done = {}

        def taps(ref, rows, after):
            cur = pltpu.bitcast(ref[J + 1, rows, :], u32)
            prv = pltpu.bitcast(ref[J, rows, :], u32)
            if after is not None:
                z = pltpu.bitcast(after, u32) & zero
                cur, prv = cur | z, prv | z
            res = []
            for w in range(TAPS):
                sh = DIL * w
                z = cur if w == 0 else jnp.where(lane16 < sh, pltpu.roll(prv, sh, 1), pltpu.roll(cur, sh, 1))
                res.append(pltpu.bitcast(z, bf).astype(f32))
            return res

        def attn_a(g):
            for h in range(4 * g, 4 * g + 4):
                rows = slice(DH * h, DH * (h + 1))
                q = aqT[J, rows, :].astype(f32)
                logits = []
                for w, kf in enumerate(taps(akT, rows, done.get(h - A_CHAIN[kind]))):
                    l = jnp.sum(q * kf, axis=0, keepdims=True)
                    logits.append(l if w == 0 else jnp.where(tap_ok[w], l, NEG))
                m = logits[0]
                for l in logits[1:]:
                    m = jnp.maximum(m, l)
                ps = [jnp.exp2(l - m) for l in logits]
                tot = ps[0]
                for p in ps[1:]:
                    tot = tot + p
                r = _recip(tot)
                acc = None
                for p, vf in zip(ps, taps(avT, rows, logits[0])):
                    t = (p * r) * vf
                    acc = t if acc is None else acc + t
                aoT[J, rows, :] = acc.astype(bf)
                done[h] = acc[0:1]

        if doO:
            oa = aoT[Jo].T
            ob = boT[Jo].T

        def out_a(lo, n):
            o[:, lo:lo + n] = _dot(oa, pltpu.bitcast(awo32[:, lo:lo + n], bf)).astype(bf)

        def out_b(lo, n):
            o[:, D + lo:D + lo + n] = _dot(ob, pltpu.bitcast(bwo32[:, lo:lo + n], bf)).astype(bf)

        lists = []
        if doP:
            lists += [[(fn, lo, 128) for lo in range(0, n * D, 128)] for fn, n in ((proj_a, 3), (proj_b, 2), (proj_bv, 1))]
        if kind == "O":
            piece, seq = 2 * D // OSPLIT, []
            for c in range(0, 2 * D, 128):
                seq.append((out_a, c, 128) if c < D else (out_b, c - D, 128))
                if (c + 128) % piece == 0:
                    seq.append((lambda lo, n: o_last(lo, n).start(), c + 128 - piece, piece))
            lists.append(seq)
        elif doO:
            lists += [[(fn, lo, 128) for lo in range(0, D, 128)] for fn in (out_a, out_b)]
        order = ORDER[kind]
        nr = order.count("r")
        slots = [[] for _ in range(nr * 8)]
        for frac, task in sorted((((i + 0.5) / len(l), t) for l in lists for i, t in enumerate(l)), key=lambda z: z[0]):
            slots[min(int(frac * nr * 8), nr * 8 - 1)].append(task)
        offs = [0] + [int(t[2:]) for t in order if t != "r"]
        scores, probs = {}, {}
        for i in range(-max(offs), 8 - min(offs)):
            k = 0
            for tok in order:
                if tok == "r":
                    if 0 <= i < 8:
                        for fn, lo, n in slots[nr * i + k]:
                            fn(lo, n)
                    k += 1
                    continue
                g = i + int(tok[2:])
                if not 0 <= g < 8:
                    continue
                if tok[:2] == "qB":
                    scores[g] = qk_b(g)
                elif tok[:2] == "sB":
                    probs[g] = softmax_b(scores.pop(g))
                elif tok[:2] == "pB":
                    pv_b(g, probs.pop(g))
                else:
                    attn_a(g)
        if kind == "PT":
            wait(wo_copies())
            awo32[...] = pltpu.bitcast(awo[...], u32)
            bwo32[...] = pltpu.bitcast(bwo[...], u32)
        if doO and kind != "O":
            o_copy(s).start()

    first_step()
    step(jnp.int32(1), "PT")
    lax.fori_loop(2, NT - 1, lambda s, c: (step(s, "PTO"), c)[1], 0)
    lax.fori_loop(NT - 1, NT + 1, lambda s, c: (step(s, "TO"), c)[1], 0)
    step(jnp.int32(NT + 1), "O")
    o_copy(NT).wait()
    for lo in range(0, 2 * D, 2 * D // OSPLIT):
        o_last(lo, 2 * D // OSPLIT).wait()


@jax.jit
def pallas_concat_heads__sliding_local_dilated__sliding_block__prompt_kernel(
    A_x: jax.Array,
    A_wqkv: jax.Array,
    A_wo: jax.Array,
    B_x: jax.Array,
    B_wqkv: jax.Array,
    B_wo: jax.Array,
):
    hbm = pl.BlockSpec(memory_space=pl.ANY)
    vmem = pltpu.VMEM
    out = pl.pallas_call(
        _kernel,
        in_specs=[hbm] * 6,
        out_specs=hbm,
        out_shape=jax.ShapeDtypeStruct((S, 2 * D), bf),
        scratch_shapes=[
            vmem((D, 3 * D), bf), vmem((D, D), bf), vmem((D, 3 * D), bf), vmem((D, D), bf),
            vmem((3 * D // 2, D), u32), vmem((D // 2, D), u32),
            vmem((D // 2, 2 * D), u32), vmem((D // 2, D), u32), vmem((D // 2, D), u32),
            vmem((3, T, D), bf), vmem((3, T, D), bf), vmem((2, T, 2 * D), bf),
            vmem((NT, D, T), bf), vmem((NT + 1, D, T), bf), vmem((NT + 1, D, T), bf),
            vmem((NT, D, T), bf),
            vmem((S, D), bf), vmem((S + 2 * T, D), bf),
            vmem((NT + 2, D, T), bf), vmem((NT, D, T), bf),
            vmem((8, T), u32),
            pltpu.SemaphoreType.DMA((4,)), pltpu.SemaphoreType.DMA((3,)), pltpu.SemaphoreType.DMA((2,)),
        ],
        compiler_params=pltpu.CompilerParams(vmem_limit_bytes=100 * 1024 * 1024),
    )(A_x[0], A_wqkv, A_wo, B_x[0], B_wqkv, B_wo)
    return out[None]
```
